```python
import os as _os
_os.environ.setdefault("JAX_PLATFORMS", "cpu")
import jax
import jax.numpy as jnp

def _softmax(x, axis=-1):
    return jax.nn.softmax(x, axis=axis)
def _gelu(x):
    return jax.nn.gelu(x, approximate=True)
def _silu(x):
    return jax.nn.silu(x)
def _sigmoid(x):
    return jax.nn.sigmoid(x)
def _layernorm(x, axis=-1, eps=1e-5):
    m = jnp.mean(x, axis=axis, keepdims=True)
    v = jnp.var(x, axis=axis, keepdims=True)
    return (x - m) / jnp.sqrt(v + eps)
def _scatter_add(tgt, idx, src, axis=0):
    return tgt.at[idx].add(src)
def _segment_sum(src, seg, n):
    return jax.ops.segment_sum(src, seg, n)
class _Rng:
    def __init__(self, key):
        self._k = key
    def _next(self):
        self._k, sub = jax.random.split(self._k)
        return sub
    def normal(self, shape):
        return jax.random.normal(self._next(), shape, dtype=jnp.bfloat16)
    def randint(self, lo, hi, shape):
        return jax.random.randint(self._next(), shape, lo, hi, dtype=jnp.int32)
    def uniform(self, shape, lo=0.0, hi=1.0):
        return jax.random.uniform(self._next(), shape, jnp.bfloat16, lo, hi)
    def permutation(self, n):
        return jax.random.permutation(self._next(), n)


kernel_name = 'sequential_preLN__softmax_full_mha__glu_gated_swiglu__prompt'

def setup_inputs():
    _rng = _Rng(jax.random.key(int.from_bytes(__import__("os").urandom(4), "little")))
    _w = (lambda a: (lambda t: t.astype(jnp.bfloat16) if jnp.issubdtype(t.dtype, jnp.floating) else t)(jnp.asarray(a)))
    def _A_setup():
        B, S, D = 1, 2048, 640
        return {
            "x": _w((lambda *s: _rng.normal(s) * 0.05)(B, S, D)),
            "wqkv": _w((lambda *s: _rng.normal(s) * 0.05)(D, 3 * D)),
            "wo": _w((lambda *s: _rng.normal(s) * 0.05)(D, D)),
        }
    _A_in = _A_setup()

    def _B_setup():
        B, S, D, F = 1, 2048, 640, 1728
        return {
            "x": _w((lambda *s: _rng.normal(s) * 0.05)(B, S, D)),
            "w1": _w((lambda *s: _rng.normal(s) * 0.05)(D, F) * (2.0 / D) ** 0.5),
            "w3": _w((lambda *s: _rng.normal(s) * 0.05)(D, F) * (2.0 / D) ** 0.5),
            "w2": _w((lambda *s: _rng.normal(s) * 0.05)(F, D) * (2.0 / F) ** 0.5),
        }
    _B_in = _B_setup()

    return {
        "A_x": _A_in["x"],
        "A_wqkv": _A_in["wqkv"],
        "A_wo": _A_in["wo"],
        "B_x": _B_in["x"],
        "B_w1": _B_in["w1"],
        "B_w3": _B_in["w3"],
        "B_w2": _B_in["w2"],
    }

def reference(A_x, A_wqkv, A_wo, B_x, B_w1, B_w3, B_w2):
    def _A_ref(x, wqkv, wo):
        B, S, D = x.shape
        H = 32; Dh = D // H
        qkv = (lambda x, *d: x.transpose(*d))((x @ wqkv).reshape(B, S, 3, H, Dh), 2, 0, 3, 1, 4)
        q, k, v = qkv[0], qkv[1], qkv[2]
        scale = Dh ** -0.5
        scores = jnp.einsum("bhqd,bhkd->bhqk", q, k) * scale
        p = _softmax(scores, axis=-1)
        o = jnp.einsum("bhqk,bhkd->bhqd", p, v)
        return (lambda x, *d: x.transpose(*d))(o, 0, 2, 1, 3).reshape(B, S, D) @ wo

    def _B_ref(x, w1, w3, w2):
        gate = jnp.einsum("bsd,df->bsf", x, w1)
        up = jnp.einsum("bsd,df->bsf", x, w3)
        h = _silu(gate) * up
        out = jnp.einsum("bsf,fd->bsd", h, w2)
        return out

    x = A_x
    h = x + _A_ref(_layernorm(x, axis=-1), A_wqkv, A_wo)
    h2 = h + _B_ref(_layernorm(h, axis=-1), B_w1, B_w3, B_w2)
    return h2
```

```python
import jax
import jax.numpy as jnp
from jax import lax
from jax.experimental import pallas as pl
from jax.experimental.pallas import tpu as pltpu

S, D, H, DH, F = 2048, 640, 32, 20, 1728
EPS = 1e-5
LOG2E = 1.4426950408889634
QSCALE = (DH ** -0.5) * LOG2E
WSTART = (0, 120, 240, 360, 480, 512)

f32, bf16 = jnp.float32, jnp.bfloat16

BM1 = 256
BMQ = 512
LNR = 64
XPARTS = ((0, 512), (512, 1024), (1024, 2048))
BQ = 512
BK = 128
ROT = 2
BM3 = 256
FCH = (512, 512, 512, 128)
LNPOS, MMPOS = 1, 2


def _ln(v):
    mu = jnp.mean(v, axis=-1, keepdims=True)
    c = v - mu
    var = jnp.mean(c * c, axis=-1, keepdims=True)
    return c * lax.rsqrt(var + EPS)


def _dot(a, b):
    return jnp.dot(a, b, preferred_element_type=f32)


def _nt(a, b):
    return lax.dot_general(a, b, (((1,), (1,)), ((), ())), preferred_element_type=f32)


def _tn(a, b):
    return lax.dot_general(a, b, (((0,), (0,)), ((), ())), preferred_element_type=f32)


def _rows(i, n):
    return pl.ds(i * n, n)


def _kernel(x_hbm, wqkv_hbm, wo_hbm, w1t_hbm, w3t_hbm, w2_hbm, out_hbm,
            x_v, wq_v, wk_v, wv_v, wo_v, w1t_v, w3t_v, w2_v,
            wqT_v, wvT_v, xn_v, kw_v, qtw_v, vt_v, ot_v, s0_v, qz0_v, out_v, sem_in, sem_out):
    cp_wk = pltpu.make_async_copy(wqkv_hbm.at[:, pl.ds(D, D)], wk_v, sem_in.at[0])
    cp_wq = pltpu.make_async_copy(wqkv_hbm.at[:, pl.ds(0, D)], wq_v, sem_in.at[1])
    cp_wv = pltpu.make_async_copy(wqkv_hbm.at[:, pl.ds(2 * D, D)], wv_v, sem_in.at[2])
    cp_x = [pltpu.make_async_copy(x_hbm.at[pl.ds(r0, r1 - r0)], x_v.at[pl.ds(r0, r1 - r0)], sem_in.at[3 + n])
            for n, (r0, r1) in enumerate(XPARTS)]
    nx = len(XPARTS)
    cp_wo = pltpu.make_async_copy(wo_hbm, wo_v, sem_in.at[3 + nx])
    cp_w1 = pltpu.make_async_copy(w1t_hbm, w1t_v, sem_in.at[4 + nx])
    cp_w3 = pltpu.make_async_copy(w3t_hbm, w3t_v, sem_in.at[5 + nx])
    cp_w2 = pltpu.make_async_copy(w2_hbm, w2_v, sem_in.at[6 + nx])
    for cp in (cp_x[0], cp_wk, cp_wq, cp_wv, *cp_x[1:], cp_wo, cp_w1, cp_w3, cp_w2):
        cp.start()

    waited = set()

    def ln_block(i):
        for n, (r0, _) in enumerate(XPARTS):
            if r0 < (i + 1) * BM1 and n not in waited:
                cp_x[n].wait()
                waited.add(n)
        for r in range(i * BM1, (i + 1) * BM1, LNR):
            xn_v[r:r + LNR, :] = _ln(x_v[r:r + LNR, :].astype(f32)).astype(bf16)

    def k_mm(i):
        return _dot(xn_v[_rows(i, BM1), :], wk_v[...])

    def k_post(i, k):
        kb = k.astype(bf16)
        for g, w0 in enumerate(WSTART):
            kw_v[g, _rows(i, BM1), :] = kb[:, w0:w0 + 128]

    def qt_block(b):
        qt = _nt(wqT_v[...], xn_v[_rows(b, BMQ), :]) * QSCALE
        for g, w0 in enumerate(WSTART):
            qtw_v[g, :, _rows(b, BMQ)] = qt[w0:w0 + 128, :].astype(bf16)

    def vt_block(b):
        vt_v[:, _rows(b, BMQ)] = _nt(wvT_v[...], xn_v[_rows(b, BMQ), :])

    kpb = BMQ // BM1
    ln_block(0)
    cp_wk.wait()
    ks = {0: k_mm(0)}
    ln_block(1)
    cp_wq.wait()
    ks[1] = k_mm(1)
    wqT_v[...] = wq_v[...].T
    k_post(0, ks.pop(0))
    cp_wv.wait()
    for b in range(S // BMQ):
        if b > 0:
            for i in range(b * kpb, (b + 1) * kpb):
                ks[i] = k_mm(i)
        qt_block(b)
        if b == 0:
            wvT_v[...] = wv_v[...].T
        for i in range(b * kpb, (b + 1) * kpb):
            if i in ks:
                k_post(i, ks.pop(i))
        if (b + 1) * BMQ < S:
            for i in range((b + 1) * kpb, (b + 2) * kpb):
                ln_block(i)
        vt_block(b)

    nq, nk = S // BQ, S // BK
    rows = lax.broadcasted_iota(jnp.int32, (128, BQ), 0)
    sub24 = lax.broadcasted_iota(jnp.int32, (24, BK), 0)
    sub8 = lax.broadcasted_iota(jnp.int32, (8, BQ), 0)

    def pair_geom(p):
        g = p // 3
        return g, 40 * p - jnp.where(g == 5, 512, 120 * g), 40 * p

    def make_qz(geom, qb, e):
        g, off, _ = geom
        lo = off + DH * e
        qw = qtw_v[g, :, _rows(qb, BQ)]
        return jnp.where((rows >= lo) & (rows < lo + DH), qw, jnp.zeros_like(qw))

    def qk_tile(geom, qz, j):
        return _dot(kw_v[geom[0], _rows(j, BK), :], qz)

    def attn_pair(p, geom):
        v0 = pl.multiple_of(geom[2], 8)
        geom_next = pair_geom(jnp.minimum(p + 1, H // 2 - 1))
        units = [(qb, e) for qb in range(nq) for e in range(2)]
        steps = [(u, j) for u in range(len(units)) for j in range(nk)]
        T = len(steps)
        ss = {t: s0_v[t] for t in range(ROT)}
        qz = {0: qz0_v[...]}
        ps, al = {}, {}
        st = {"m": None, "acc": None, "even": None}

        def scores(t):
            u, j = steps[t]
            if u not in qz:
                qz[u] = make_qz(geom, *units[u])
            return qk_tile(geom, qz[u], j)

        def softmax(t):
            _, j = steps[t]
            s = ss.pop(t)
            mb = jnp.max(s, axis=0, keepdims=True)
            if j == 0:
                m_new, al[t] = mb, None
            else:
                m_new = jnp.maximum(st["m"], mb)
                al[t] = jnp.exp2(st["m"] - m_new)
            ps[t] = jnp.exp2(s - m_new)
            st["m"] = m_new

        def accum(t):
            u, j = steps[t]
            qb, e = units[u]
            vt = vt_v[pl.ds(v0 + 16 * e, 24), _rows(j, BK)]
            vt = jnp.where((sub24 >= DH) if e == 0 else (sub24 < 4), 1.0, vt)
            o = _dot(vt, ps.pop(t))
            a = al.pop(t)
            st["acc"] = o if a is None else a * st["acc"] + o
            if j == nk - 1:
                acc = st["acc"]
                if e == 0:
                    st["even"] = acc * (1.0 / acc[DH:DH + 1, :])
                else:
                    odd = acc * (1.0 / acc[0:1, :])
                    even = st["even"]
                    mid = jnp.where(sub8 < 4, even[16:24, :], odd[0:8, :])
                    ot_v[pl.ds(v0, 40), _rows(qb, BQ)] = jnp.concatenate(
                        [even[0:16, :], mid, odd[8:24, :]], axis=0)

        qz_next = None
        for t in range(T + 1):
            if ROT <= t + 1 < T:
                ss[t + 1] = scores(t + 1)
            elif t + 1 >= T:
                if qz_next is None:
                    qz_next = make_qz(geom_next, 0, 0)
                    qz0_v[...] = qz_next
                s0_v[t + 1 - T] = qk_tile(geom_next, qz_next, t + 1 - T)
            if t < T:
                softmax(t)
            if t >= 1:
                accum(t - 1)
        return geom_next

    geom0 = pair_geom(jnp.int32(0))
    qz0 = make_qz(geom0, 0, 0)
    qz0_v[...] = qz0
    for t in range(ROT):
        s0_v[t] = qk_tile(geom0, qz0, t)
    lax.fori_loop(0, H // 2, attn_pair, geom0)

    for cp in (cp_wo, cp_w1, cp_w3, cp_w2):
        cp.wait()
    nb3 = S // BM3
    FR = sum(FCH)
    chunks, c0 = [], 0
    for cw in FCH:
        chunks.append((c0, cw))
        c0 += cw
    order = [len(chunks)] + list(range(len(chunks)))[::-1]

    def proj_mm(i):
        ot = ot_v[:, _rows(i, BM3)].astype(bf16)
        return x_v[_rows(i, BM3), :].astype(f32) + _tn(ot, wo_v[...])

    def gate_up(hn, c):
        if c < len(chunks):
            c0, cw = chunks[c]
            return _nt(hn, w1t_v[c0:c0 + cw, :]), _nt(hn, w3t_v[c0:c0 + cw, :])
        r = _nt(hn, jnp.concatenate([w1t_v[FR:F, :], w3t_v[FR:F, :]], axis=0))
        return r, pltpu.roll(r, F - FR, 1)

    def down(c, gt, up):
        a = gt * jax.nn.sigmoid(gt) * up
        if c < len(chunks):
            c0, cw = chunks[c]
            return _dot(a.astype(bf16), w2_v[c0:c0 + cw, :])
        return _dot(a[:, 0:F - FR].astype(bf16), w2_v[FR:F, :])

    hs = {0: proj_mm(0), 1: proj_mm(1)}
    hn = _ln(hs[0]).astype(bf16)
    nxt = gate_up(hn, order[0])
    for i in range(nb3):
        acc = hs.pop(i)
        hn_next = None
        for n, c in enumerate(order):
            cur = nxt
            if n + 1 < len(order):
                nxt = gate_up(hn, order[n + 1])
            elif i + 1 < nb3:
                nxt = gate_up(hn_next, order[0])
            if n == LNPOS and i + 1 < nb3:
                hn_next = _ln(hs[i + 1]).astype(bf16)
            if n == MMPOS and i + 2 < nb3:
                hs[i + 2] = proj_mm(i + 2)
            acc = acc + down(c, *cur)
        out_v[_rows(i, BM3), :] = acc.astype(bf16)
        pltpu.make_async_copy(out_v.at[_rows(i, BM3)], out_hbm.at[_rows(i, BM3)], sem_out.at[i]).start()
        hn = hn_next
    for i in range(nb3):
        pltpu.make_async_copy(out_v.at[_rows(i, BM3)], out_hbm.at[_rows(i, BM3)], sem_out.at[i]).wait()


@jax.jit
def pallas_sequential_preLN__softmax_full_mha__glu_gated_swiglu__prompt_kernel(A_x, A_wqkv, A_wo, B_x, B_w1, B_w3, B_w2):
    del B_x
    hbm = pl.BlockSpec(memory_space=pltpu.HBM)
    out = pl.pallas_call(
        _kernel,
        out_shape=jax.ShapeDtypeStruct((S, D), bf16),
        in_specs=[hbm] * 6,
        out_specs=hbm,
        scratch_shapes=[
            pltpu.VMEM((S, D), bf16),
            pltpu.VMEM((D, D), bf16),
            pltpu.VMEM((D, D), bf16),
            pltpu.VMEM((D, D), bf16),
            pltpu.VMEM((D, D), bf16),
            pltpu.VMEM((F, D), bf16),
            pltpu.VMEM((F, D), bf16),
            pltpu.VMEM((F, D), bf16),
            pltpu.VMEM((D, D), bf16),
            pltpu.VMEM((D, D), bf16),
            pltpu.VMEM((S, D), bf16),
            pltpu.VMEM((6, S, 128), bf16),
            pltpu.VMEM((6, 128, S), bf16),
            pltpu.VMEM((D, S), f32),
            pltpu.VMEM((D, S), f32),
            pltpu.VMEM((ROT, BK, BQ), f32),
            pltpu.VMEM((128, BQ), bf16),
            pltpu.VMEM((S, D), bf16),
            pltpu.SemaphoreType.DMA((7 + len(XPARTS),)),
            pltpu.SemaphoreType.DMA((S // BM3,)),
        ],
        compiler_params=pltpu.CompilerParams(vmem_limit_bytes=100 * 1024 * 1024),
        name="fused_block",
    )(A_x.reshape(S, D), A_wqkv, A_wo, B_w1.T, B_w3.T, B_w2)
    return out.reshape(1, S, D)
```

```python
import jax
import jax.numpy as jnp
from jax import lax
from jax.experimental import pallas as pl
from jax.experimental.pallas import tpu as pltpu

S, D, H, DH, F = 2048, 640, 32, 20, 1728
EPS = 1e-5
LOG2E = 1.4426950408889634
QSCALE = (DH ** -0.5) * LOG2E
WSTART = (0, 120, 240, 360, 480, 512)

f32, bf16 = jnp.float32, jnp.bfloat16

BM1 = 256
BMQ = 512
LNR = 64
XPARTS = ((0, 512), (512, 1024), (1024, 2048))
BQ = 512
BK = 128
ROT = 2
PACE_ROW = 8
PACE_SKIP = (0, 1)
BM3 = 256
FCH = (512, 512, 512, 128)
LNPOS, MMPOS = 1, 2


def _ln(v):
    mu = jnp.mean(v, axis=-1, keepdims=True)
    c = v - mu
    var = jnp.mean(c * c, axis=-1, keepdims=True)
    return c * lax.rsqrt(var + EPS)


def _dot(a, b):
    return jnp.dot(a, b, preferred_element_type=f32)


def _nt(a, b):
    return lax.dot_general(a, b, (((1,), (1,)), ((), ())), preferred_element_type=f32)


def _tn(a, b):
    return lax.dot_general(a, b, (((0,), (0,)), ((), ())), preferred_element_type=f32)


def _rows(i, n):
    return pl.ds(i * n, n)


def _kernel(x_hbm, wqkv_hbm, wo_hbm, w1t_hbm, w3t_hbm, w2_hbm, out_hbm,
            x_v, wq_v, wk_v, wv_v, wo_v, w1t_v, w3t_v, w2_v,
            wqT_v, wvT_v, xn_v, kw_v, qt_v, vt_v, ot_v, s0_v, qz0_v, out_v, sem_in, sem_out):
    cp_wk = pltpu.make_async_copy(wqkv_hbm.at[:, pl.ds(D, D)], wk_v, sem_in.at[0])
    cp_wq = pltpu.make_async_copy(wqkv_hbm.at[:, pl.ds(0, D)], wq_v, sem_in.at[1])
    cp_wv = pltpu.make_async_copy(wqkv_hbm.at[:, pl.ds(2 * D, D)], wv_v, sem_in.at[2])
    cp_x = [pltpu.make_async_copy(x_hbm.at[pl.ds(r0, r1 - r0)], x_v.at[pl.ds(r0, r1 - r0)], sem_in.at[3 + n])
            for n, (r0, r1) in enumerate(XPARTS)]
    nx = len(XPARTS)
    cp_wo = pltpu.make_async_copy(wo_hbm, wo_v, sem_in.at[3 + nx])
    cp_w1 = pltpu.make_async_copy(w1t_hbm, w1t_v, sem_in.at[4 + nx])
    cp_w3 = pltpu.make_async_copy(w3t_hbm, w3t_v, sem_in.at[5 + nx])
    cp_w2 = pltpu.make_async_copy(w2_hbm, w2_v, sem_in.at[6 + nx])
    for cp in (cp_x[0], cp_wk, cp_wq, cp_wv, *cp_x[1:], cp_wo, cp_w1, cp_w3, cp_w2):
        cp.start()

    waited = set()

    def ln_block(i):
        for n, (r0, _) in enumerate(XPARTS):
            if r0 < (i + 1) * BM1 and n not in waited:
                cp_x[n].wait()
                waited.add(n)
        for r in range(i * BM1, (i + 1) * BM1, LNR):
            xn_v[r:r + LNR, :] = _ln(x_v[r:r + LNR, :].astype(f32)).astype(bf16)

    def k_mm(i):
        return _dot(xn_v[_rows(i, BM1), :], wk_v[...])

    def k_post(i, k):
        kb = k.astype(bf16)
        for g, w0 in enumerate(WSTART):
            kw_v[g, _rows(i, BM1), :] = kb[:, w0:w0 + 128]

    def qt_block(b):
        qt = _nt(wqT_v[...], xn_v[_rows(b, BMQ), :]) * QSCALE
        qt_v[:, _rows(b, BMQ)] = qt

    def vt_block(b):
        vt_v[:, _rows(b, BMQ)] = _nt(wvT_v[...], xn_v[_rows(b, BMQ), :])

    kpb = BMQ // BM1
    ln_block(0)
    cp_wk.wait()
    ks = {0: k_mm(0)}
    ln_block(1)
    cp_wq.wait()
    ks[1] = k_mm(1)
    wqT_v[...] = wq_v[...].T
    k_post(0, ks.pop(0))
    cp_wv.wait()
    for b in range(S // BMQ):
        if b > 0:
            for i in range(b * kpb, (b + 1) * kpb):
                ks[i] = k_mm(i)
        qt_block(b)
        if b == 0:
            wvT_v[...] = wv_v[...].T
        for i in range(b * kpb, (b + 1) * kpb):
            if i in ks:
                k_post(i, ks.pop(i))
        if (b + 1) * BMQ < S:
            for i in range((b + 1) * kpb, (b + 2) * kpb):
                ln_block(i)
        vt_block(b)

    nq, nk = S // BQ, S // BK
    rows = lax.broadcasted_iota(jnp.int32, (128, BQ), 0)
    sub24 = lax.broadcasted_iota(jnp.int32, (24, BK), 0)
    sub8 = lax.broadcasted_iota(jnp.int32, (8, BQ), 0)

    def pair_geom(p):
        g = p // 3
        w0 = jnp.where(g == 5, WSTART[5], 120 * g)
        return g, 40 * p - w0, 40 * p

    def make_qz(geom, qb, e):
        _, off, v0 = geom
        lo = off + DH * e
        qw = qt_v[pl.ds(pl.multiple_of(v0 - off, 8), 128), _rows(qb, BQ)]
        return jnp.where((rows >= lo) & (rows < lo + DH), qw, 0.0).astype(bf16)

    def qk_tile(geom, qz, j):
        return _dot(kw_v[geom[0], _rows(j, BK), :], qz)

    def attn_pair(p, geom):
        v0 = pl.multiple_of(geom[2], 8)
        geom_next = pair_geom(jnp.minimum(p + 1, H // 2 - 1))
        units = [(qb, e) for qb in range(nq) for e in range(2)]
        steps = [(u, j) for u in range(len(units)) for j in range(nk)]
        T = len(steps)
        ss = {t: s0_v[t] for t in range(ROT)}
        qz = {0: qz0_v[...]}
        ps, al = {}, {}
        st = {"m": None, "acc": None, "even": None}

        def scores(t):
            u, j = steps[t]
            if u not in qz:
                qz[u] = make_qz(geom, *units[u])
            return qk_tile(geom, qz[u], j)

        def softmax(t):
            _, j = steps[t]
            s = ss.pop(t)
            mb = jnp.max(s, axis=0, keepdims=True)
            if j == 0:
                m_new, al[t] = mb, None
            else:
                m_new = jnp.maximum(st["m"], mb)
                al[t] = jnp.exp2(st["m"] - m_new)
            st["m"] = m_new
            if t + 1 in ss and j not in PACE_SKIP:
                nxt = ss[t + 1][PACE_ROW:PACE_ROW + 8, :]
                m_new = jnp.where(nxt < -jnp.inf, nxt, jnp.broadcast_to(m_new, (8, BQ)))
                m_new = jnp.concatenate([m_new] * (BK // 8), axis=0)
            ps[t] = jnp.exp2(s - m_new)

        def accum(t):
            u, j = steps[t]
            qb, e = units[u]
            vt = vt_v[pl.ds(v0 + 16 * e, 24), _rows(j, BK)]
            vt = jnp.where((sub24 >= DH) if e == 0 else (sub24 < 4), 1.0, vt)
            o = _dot(vt, ps.pop(t))
            a = al.pop(t)
            st["acc"] = o if a is None else a * st["acc"] + o
            if j == nk - 1:
                acc = st["acc"]
                if e == 0:
                    st["even"] = acc * (1.0 / acc[DH:DH + 1, :])
                else:
                    odd = acc * (1.0 / acc[0:1, :])
                    even = st["even"]
                    mid = jnp.where(sub8 < 4, even[16:24, :], odd[0:8, :])
                    ot_v[pl.ds(v0, 40), _rows(qb, BQ)] = jnp.concatenate(
                        [even[0:16, :], mid, odd[8:24, :]], axis=0)

        qz_next = None
        for t in range(T + 1):
            if ROT <= t + 1 < T:
                ss[t + 1] = scores(t + 1)
            elif t + 1 >= T:
                if qz_next is None:
                    qz_next = make_qz(geom_next, 0, 0)
                    qz0_v[...] = qz_next
                ss[t + 1] = qk_tile(geom_next, qz_next, t + 1 - T)
                s0_v[t + 1 - T] = ss[t + 1]
            if t < T:
                softmax(t)
            if t >= 1:
                accum(t - 1)
        return geom_next

    geom0 = pair_geom(jnp.int32(0))
    qz0 = make_qz(geom0, 0, 0)
    qz0_v[...] = qz0
    for t in range(ROT):
        s0_v[t] = qk_tile(geom0, qz0, t)
    lax.fori_loop(0, H // 2, attn_pair, geom0)

    for cp in (cp_wo, cp_w1, cp_w3, cp_w2):
        cp.wait()
    nb3 = S // BM3
    FR = sum(FCH)
    chunks, c0 = [], 0
    for cw in FCH:
        chunks.append((c0, cw))
        c0 += cw
    order = [len(chunks)] + list(range(len(chunks)))[::-1]

    def proj_mm(i):
        ot = ot_v[:, _rows(i, BM3)].astype(bf16)
        return x_v[_rows(i, BM3), :].astype(f32) + _tn(ot, wo_v[...])

    def gate_up(hn, c):
        if c < len(chunks):
            c0, cw = chunks[c]
            return _nt(hn, w1t_v[c0:c0 + cw, :]), _nt(hn, w3t_v[c0:c0 + cw, :])
        r = _nt(hn, jnp.concatenate([w1t_v[FR:F, :], w3t_v[FR:F, :]], axis=0))
        return r, pltpu.roll(r, F - FR, 1)

    def down(c, gt, up):
        a = gt * jax.nn.sigmoid(gt) * up
        if c < len(chunks):
            c0, cw = chunks[c]
            return _dot(a.astype(bf16), w2_v[c0:c0 + cw, :])
        return _dot(a[:, 0:F - FR].astype(bf16), w2_v[FR:F, :])

    hs = {0: proj_mm(0), 1: proj_mm(1)}
    hn = _ln(hs[0]).astype(bf16)
    nxt = gate_up(hn, order[0])
    for i in range(nb3):
        acc = hs.pop(i)
        hn_next = None
        for n, c in enumerate(order):
            cur = nxt
            if n + 1 < len(order):
                nxt = gate_up(hn, order[n + 1])
            elif i + 1 < nb3:
                nxt = gate_up(hn_next, order[0])
            if n == LNPOS and i + 1 < nb3:
                hn_next = _ln(hs[i + 1]).astype(bf16)
            if n == MMPOS and i + 2 < nb3:
                hs[i + 2] = proj_mm(i + 2)
            acc = acc + down(c, *cur)
        out_v[_rows(i, BM3), :] = acc.astype(bf16)
        pltpu.make_async_copy(out_v.at[_rows(i, BM3)], out_hbm.at[_rows(i, BM3)], sem_out.at[i]).start()
        hn = hn_next
    for i in range(nb3):
        pltpu.make_async_copy(out_v.at[_rows(i, BM3)], out_hbm.at[_rows(i, BM3)], sem_out.at[i]).wait()


@jax.jit
def pallas_sequential_preLN__softmax_full_mha__glu_gated_swiglu__prompt_kernel(A_x, A_wqkv, A_wo, B_x, B_w1, B_w3, B_w2):
    del B_x
    hbm = pl.BlockSpec(memory_space=pltpu.HBM)
    out = pl.pallas_call(
        _kernel,
        out_shape=jax.ShapeDtypeStruct((S, D), bf16),
        in_specs=[hbm] * 6,
        out_specs=hbm,
        scratch_shapes=[
            pltpu.VMEM((S, D), bf16),
            pltpu.VMEM((D, D), bf16),
            pltpu.VMEM((D, D), bf16),
            pltpu.VMEM((D, D), bf16),
            pltpu.VMEM((D, D), bf16),
            pltpu.VMEM((F, D), bf16),
            pltpu.VMEM((F, D), bf16),
            pltpu.VMEM((F, D), bf16),
            pltpu.VMEM((D, D), bf16),
            pltpu.VMEM((D, D), bf16),
            pltpu.VMEM((S, D), bf16),
            pltpu.VMEM((6, S, 128), bf16),
            pltpu.VMEM((D, S), f32),
            pltpu.VMEM((D, S), f32),
            pltpu.VMEM((D, S), f32),
            pltpu.VMEM((ROT, BK, BQ), f32),
            pltpu.VMEM((128, BQ), bf16),
            pltpu.VMEM((S, D), bf16),
            pltpu.SemaphoreType.DMA((7 + len(XPARTS),)),
            pltpu.SemaphoreType.DMA((S // BM3,)),
        ],
        compiler_params=pltpu.CompilerParams(vmem_limit_bytes=100 * 1024 * 1024),
        name="fused_block",
    )(A_x.reshape(S, D), A_wqkv, A_wo, B_w1.T, B_w3.T, B_w2)
    return out.reshape(1, S, D)
```

```python
import jax
import jax.numpy as jnp
from jax import lax
from jax.experimental import pallas as pl
from jax.experimental.pallas import tpu as pltpu

S, D, H, DH, F = 2048, 640, 32, 20, 1728
EPS = 1e-5
LOG2E = 1.4426950408889634
QSCALE = (DH ** -0.5) * LOG2E
WSTART = (0, 120, 240, 360, 480, 512)

f32, bf16 = jnp.float32, jnp.bfloat16

BM1 = 256
BMQ = 512
LNR = 64
XPARTS = ((0, 512), (512, 1024), (1024, 2048))
BQ = 512
BK = 128
ROT = 2
PACE_ROW = 8
PACE_SKIP = (0, 1)
PACE_FREE = 8
BM3 = 256
FCH = (512, 512, 512, 128)
LNPOS, MMPOS = 1, 2


def _ln(v):
    mu = jnp.mean(v, axis=-1, keepdims=True)
    c = v - mu
    var = jnp.mean(c * c, axis=-1, keepdims=True)
    return c * lax.rsqrt(var + EPS)


def _dot(a, b):
    return jnp.dot(a, b, preferred_element_type=f32)


def _nt(a, b):
    return lax.dot_general(a, b, (((1,), (1,)), ((), ())), preferred_element_type=f32)


def _tn(a, b):
    return lax.dot_general(a, b, (((0,), (0,)), ((), ())), preferred_element_type=f32)


def _rows(i, n):
    return pl.ds(i * n, n)


def _kernel(x_hbm, wqkv_hbm, wo_hbm, w1t_hbm, w3t_hbm, w2_hbm, out_hbm,
            x_v, wq_v, wk_v, wv_v, wo_v, w1t_v, w3t_v, w2_v,
            wqT_v, wvT_v, xn_v, kw_v, qt_v, vt_v, ot_v, s0_v, qz0_v, out_v, sem_in, sem_out):
    cp_wk = pltpu.make_async_copy(wqkv_hbm.at[:, pl.ds(D, D)], wk_v, sem_in.at[0])
    cp_wq = pltpu.make_async_copy(wqkv_hbm.at[:, pl.ds(0, D)], wq_v, sem_in.at[1])
    cp_wv = pltpu.make_async_copy(wqkv_hbm.at[:, pl.ds(2 * D, D)], wv_v, sem_in.at[2])
    cp_x = [pltpu.make_async_copy(x_hbm.at[pl.ds(r0, r1 - r0)], x_v.at[pl.ds(r0, r1 - r0)], sem_in.at[3 + n])
            for n, (r0, r1) in enumerate(XPARTS)]
    nx = len(XPARTS)
    cp_wo = pltpu.make_async_copy(wo_hbm, wo_v, sem_in.at[3 + nx])
    cp_w1 = pltpu.make_async_copy(w1t_hbm, w1t_v, sem_in.at[4 + nx])
    cp_w3 = pltpu.make_async_copy(w3t_hbm, w3t_v, sem_in.at[5 + nx])
    cp_w2 = pltpu.make_async_copy(w2_hbm, w2_v, sem_in.at[6 + nx])
    for cp in (cp_x[0], cp_wk, cp_wq, cp_wv, *cp_x[1:], cp_wo, cp_w1, cp_w3, cp_w2):
        cp.start()

    waited = set()

    def ln_block(i):
        for n, (r0, _) in enumerate(XPARTS):
            if r0 < (i + 1) * BM1 and n not in waited:
                cp_x[n].wait()
                waited.add(n)
        for r in range(i * BM1, (i + 1) * BM1, LNR):
            xn_v[r:r + LNR, :] = _ln(x_v[r:r + LNR, :].astype(f32)).astype(bf16)

    def k_mm(i):
        return _dot(xn_v[_rows(i, BM1), :], wk_v[...])

    def k_post(i, k):
        kb = k.astype(bf16)
        for g, w0 in enumerate(WSTART):
            kw_v[g, _rows(i, BM1), :] = kb[:, w0:w0 + 128]

    def qt_block(b):
        qt = _nt(wqT_v[...], xn_v[_rows(b, BMQ), :]) * QSCALE
        qt_v[:, _rows(b, BMQ)] = qt

    def vt_block(b):
        vt_v[:, _rows(b, BMQ)] = _nt(wvT_v[...], xn_v[_rows(b, BMQ), :])

    kpb = BMQ // BM1
    ln_block(0)
    cp_wk.wait()
    ks = {0: k_mm(0)}
    ln_block(1)
    cp_wq.wait()
    ks[1] = k_mm(1)
    wqT_v[...] = wq_v[...].T
    k_post(0, ks.pop(0))
    cp_wv.wait()
    for b in range(S // BMQ):
        nxt_ln = range((b + 1) * kpb, (b + 2) * kpb) if (b + 1) * BMQ < S else ()
        if b > 0:
            for i in range(b * kpb, (b + 1) * kpb):
                ks[i] = k_mm(i)
            for i in nxt_ln:
                ln_block(i)
        qt_block(b)
        if b == 0:
            wvT_v[...] = wv_v[...].T
        for i in range(b * kpb, (b + 1) * kpb):
            if i in ks:
                k_post(i, ks.pop(i))
        if b == 0:
            for i in nxt_ln:
                ln_block(i)
        vt_block(b)

    nq, nk = S // BQ, S // BK
    rows = lax.broadcasted_iota(jnp.int32, (128, BQ), 0)
    sub24 = lax.broadcasted_iota(jnp.int32, (24, BK), 0)
    sub8 = lax.broadcasted_iota(jnp.int32, (8, BQ), 0)

    def pair_geom(p):
        g = p // 3
        w0 = jnp.where(g == 5, WSTART[5], 120 * g)
        return g, 40 * p - w0, 40 * p

    def make_qz(geom, qb, e):
        _, off, v0 = geom
        lo = off + DH * e
        qw = qt_v[pl.ds(pl.multiple_of(v0 - off, 8), 128), _rows(qb, BQ)]
        return jnp.where((rows >= lo) & (rows < lo + DH), qw, 0.0).astype(bf16)

    def qk_tile(geom, qz, j):
        return _dot(kw_v[geom[0], _rows(j, BK), :], qz)

    def attn_pair(p, geom):
        v0 = pl.multiple_of(geom[2], 8)
        geom_next = pair_geom(jnp.minimum(p + 1, H // 2 - 1))
        units = [(qb, e) for qb in range(nq) for e in range(2)]
        steps = [(u, j) for u in range(len(units)) for j in range(nk)]
        T = len(steps)
        ss = {t: s0_v[t] for t in range(ROT)}
        qz = {0: qz0_v[...]}
        ps, al = {}, {}
        st = {"m": None, "acc": None, "even": None}

        def scores(t):
            u, j = steps[t]
            if u not in qz:
                qz[u] = make_qz(geom, *units[u])
            return qk_tile(geom, qz[u], j)

        def softmax(t):
            _, j = steps[t]
            s = ss.pop(t)
            mb = jnp.max(s, axis=0, keepdims=True)
            if j == 0:
                m_new, al[t] = mb, None
            else:
                m_new = jnp.maximum(st["m"], mb)
                al[t] = jnp.exp2(st["m"] - m_new)
            st["m"] = m_new
            if t + 1 in ss and j not in PACE_SKIP:
                nxt = ss[t + 1][PACE_ROW:PACE_ROW + 8, :]
                m8 = jnp.broadcast_to(m_new, (8, BQ))
                paced = jnp.where(nxt < -jnp.inf, nxt, m8)
                m_new = jnp.concatenate([m8] * PACE_FREE + [paced] * (BK // 8 - PACE_FREE), axis=0)
            ps[t] = jnp.exp2(s - m_new)

        def accum(t):
            u, j = steps[t]
            qb, e = units[u]
            vt = vt_v[pl.ds(v0 + 16 * e, 24), _rows(j, BK)]
            vt = jnp.where((sub24 >= DH) if e == 0 else (sub24 < 4), 1.0, vt)
            o = _dot(vt, ps.pop(t))
            a = al.pop(t)
            st["acc"] = o if a is None else a * st["acc"] + o
            if j == nk - 1:
                acc = st["acc"]
                if e == 0:
                    st["even"] = acc * (1.0 / acc[DH:DH + 1, :])
                else:
                    odd = acc * (1.0 / acc[0:1, :])
                    even = st["even"]
                    mid = jnp.where(sub8 < 4, even[16:24, :], odd[0:8, :])
                    ot_v[pl.ds(v0, 40), _rows(qb, BQ)] = jnp.concatenate(
                        [even[0:16, :], mid, odd[8:24, :]], axis=0)

        qz_next = None
        for t in range(T + 1):
            if ROT <= t + 1 < T:
                ss[t + 1] = scores(t + 1)
            elif t + 1 >= T:
                if qz_next is None:
                    qz_next = make_qz(geom_next, 0, 0)
                    qz0_v[...] = qz_next
                ss[t + 1] = qk_tile(geom_next, qz_next, t + 1 - T)
                s0_v[t + 1 - T] = ss[t + 1]
            if t < T:
                softmax(t)
            if t >= 1:
                accum(t - 1)
        return geom_next

    geom0 = pair_geom(jnp.int32(0))
    qz0 = make_qz(geom0, 0, 0)
    qz0_v[...] = qz0
    for t in range(ROT):
        s0_v[t] = qk_tile(geom0, qz0, t)
    lax.fori_loop(0, H // 2, attn_pair, geom0)

    for cp in (cp_wo, cp_w1, cp_w3, cp_w2):
        cp.wait()
    nb3 = S // BM3
    FR = sum(FCH)
    chunks, c0 = [], 0
    for cw in FCH:
        chunks.append((c0, cw))
        c0 += cw
    order = [len(chunks)] + list(range(len(chunks)))[::-1]

    def proj_mm(i):
        ot = ot_v[:, _rows(i, BM3)].astype(bf16)
        return x_v[_rows(i, BM3), :].astype(f32) + _tn(ot, wo_v[...])

    def gate_up(hn, c):
        if c < len(chunks):
            c0, cw = chunks[c]
            return _nt(hn, w1t_v[c0:c0 + cw, :]), _nt(hn, w3t_v[c0:c0 + cw, :])
        r = _nt(hn, jnp.concatenate([w1t_v[FR:F, :], w3t_v[FR:F, :]], axis=0))
        return r, pltpu.roll(r, F - FR, 1)

    def down(c, gt, up):
        a = gt * jax.nn.sigmoid(gt) * up
        if c < len(chunks):
            c0, cw = chunks[c]
            return _dot(a.astype(bf16), w2_v[c0:c0 + cw, :])
        return _dot(a[:, 0:F - FR].astype(bf16), w2_v[FR:F, :])

    hs = {0: proj_mm(0), 1: proj_mm(1)}
    hn = _ln(hs[0]).astype(bf16)
    nxt = gate_up(hn, order[0])
    for i in range(nb3):
        acc = hs.pop(i)
        hn_next = None
        for n, c in enumerate(order):
            cur = nxt
            if n + 1 < len(order):
                nxt = gate_up(hn, order[n + 1])
            elif i + 1 < nb3:
                nxt = gate_up(hn_next, order[0])
            if n == LNPOS and i + 1 < nb3:
                hn_next = _ln(hs[i + 1]).astype(bf16)
            if n == MMPOS and i + 2 < nb3:
                hs[i + 2] = proj_mm(i + 2)
            acc = acc + down(c, *cur)
        out_v[_rows(i, BM3), :] = acc.astype(bf16)
        pltpu.make_async_copy(out_v.at[_rows(i, BM3)], out_hbm.at[_rows(i, BM3)], sem_out.at[i]).start()
        hn = hn_next
    for i in range(nb3):
        pltpu.make_async_copy(out_v.at[_rows(i, BM3)], out_hbm.at[_rows(i, BM3)], sem_out.at[i]).wait()


@jax.jit
def pallas_sequential_preLN__softmax_full_mha__glu_gated_swiglu__prompt_kernel(A_x, A_wqkv, A_wo, B_x, B_w1, B_w3, B_w2):
    del B_x
    hbm = pl.BlockSpec(memory_space=pltpu.HBM)
    out = pl.pallas_call(
        _kernel,
        out_shape=jax.ShapeDtypeStruct((S, D), bf16),
        in_specs=[hbm] * 6,
        out_specs=hbm,
        scratch_shapes=[
            pltpu.VMEM((S, D), bf16),
            pltpu.VMEM((D, D), bf16),
            pltpu.VMEM((D, D), bf16),
            pltpu.VMEM((D, D), bf16),
            pltpu.VMEM((D, D), bf16),
            pltpu.VMEM((F, D), bf16),
            pltpu.VMEM((F, D), bf16),
            pltpu.VMEM((F, D), bf16),
            pltpu.VMEM((D, D), bf16),
            pltpu.VMEM((D, D), bf16),
            pltpu.VMEM((S, D), bf16),
            pltpu.VMEM((6, S, 128), bf16),
            pltpu.VMEM((D, S), f32),
            pltpu.VMEM((D, S), f32),
            pltpu.VMEM((D, S), f32),
            pltpu.VMEM((ROT, BK, BQ), f32),
            pltpu.VMEM((128, BQ), bf16),
            pltpu.VMEM((S, D), bf16),
            pltpu.SemaphoreType.DMA((7 + len(XPARTS),)),
            pltpu.SemaphoreType.DMA((S // BM3,)),
        ],
        compiler_params=pltpu.CompilerParams(vmem_limit_bytes=100 * 1024 * 1024),
        name="fused_block",
    )(A_x.reshape(S, D), A_wqkv, A_wo, B_w1.T, B_w3.T, B_w2)
    return out.reshape(1, S, D)
```
